```python
import os as _os
_os.environ.setdefault("JAX_PLATFORMS", "cpu")
import jax
import jax.numpy as jnp

def _softmax(x, axis=-1):
    return jax.nn.softmax(x, axis=axis)
def _gelu(x):
    return jax.nn.gelu(x, approximate=True)
def _silu(x):
    return jax.nn.silu(x)
def _sigmoid(x):
    return jax.nn.sigmoid(x)
def _layernorm(x, axis=-1, eps=1e-5):
    m = jnp.mean(x, axis=axis, keepdims=True)
    v = jnp.var(x, axis=axis, keepdims=True)
    return (x - m) / jnp.sqrt(v + eps)
def _scatter_add(tgt, idx, src, axis=0):
    return tgt.at[idx].add(src)
def _segment_sum(src, seg, n):
    return jax.ops.segment_sum(src, seg, n)
class _Rng:
    def __init__(self, key):
        self._k = key
    def _next(self):
        self._k, sub = jax.random.split(self._k)
        return sub
    def normal(self, shape):
        return jax.random.normal(self._next(), shape, dtype=jnp.bfloat16)
    def randint(self, lo, hi, shape):
        return jax.random.randint(self._next(), shape, lo, hi, dtype=jnp.int32)
    def uniform(self, shape, lo=0.0, hi=1.0):
        return jax.random.uniform(self._next(), shape, jnp.bfloat16, lo, hi)
    def permutation(self, n):
        return jax.random.permutation(self._next(), n)


kernel_name = 'gated_mix__linear_kernel_hedgehog__glu_gated_bilinear__prompt'

def setup_inputs():
    _rng = _Rng(jax.random.key(int.from_bytes(__import__("os").urandom(4), "little")))
    _w = (lambda a: (lambda t: t.astype(jnp.bfloat16) if jnp.issubdtype(t.dtype, jnp.floating) else t)(jnp.asarray(a)))
    def _A_setup():
        B, S, D, H = 1, 2048, 512, 32
        Dh = D // H
        return {
            "x": _w((lambda *s: _rng.normal(s) * 0.05)(B, S, D)),
            "wqkv": _w((lambda *s: _rng.normal(s) * 0.8)(D, 3 * D)),
            "w_phi": _w((lambda *s: _rng.normal(s) * 0.8)(H, Dh, Dh) * (Dh ** -0.5)),
            "wo": _w((lambda *s: _rng.normal(s) * 0.05)(D, D)),
        }
    _A_in = _A_setup()

    def _B_setup():
        B, S, D, F = 1, 2048, 512, 1792
        return {
            "x": _w((lambda *s: _rng.normal(s) * 0.05)(B, S, D)),
            "w_gate": _w((lambda *s: _rng.normal(s) * 1.6)(D, F) * (D ** -0.5)),
            "w_up": _w((lambda *s: _rng.normal(s) * 1.6)(D, F) * (D ** -0.5)),
            "w_down": _w((lambda *s: _rng.normal(s) * 1.6)(F, D) * (F ** -0.5)),
        }
    _B_in = _B_setup()

    return {
        "A_x": _A_in["x"],
        "A_wqkv": _A_in["wqkv"],
        "A_w_phi": _A_in["w_phi"],
        "A_wo": _A_in["wo"],
        "B_x": _B_in["x"],
        "B_w_gate": _B_in["w_gate"],
        "B_w_up": _B_in["w_up"],
        "B_w_down": _B_in["w_down"],
        "gate_w": _w((lambda *s: _rng.normal(s) * 0.05)(512) * 16.0),
    }

def reference(A_x, A_wqkv, A_w_phi, A_wo, B_x, B_w_gate, B_w_up, B_w_down, gate_w):
    def _A_ref(x, wqkv, w_phi, wo):
        B, S, D = x.shape
        H = 32; Dh = D // H
        qkv = (lambda x, *d: x.transpose(*d))((x @ wqkv).reshape(B, S, 3, H, Dh), 2, 0, 3, 1, 4)
        q, k, v = qkv[0], qkv[1], qkv[2]
        pq = jnp.einsum("bhsd,hdf->bhsf", q, w_phi)
        pk = jnp.einsum("bhsd,hdf->bhsf", k, w_phi)
        phi_q = jnp.concatenate([_softmax(pq, axis=-1), _softmax(-pq, axis=-1)], axis=-1)
        phi_k = jnp.concatenate([_softmax(pk, axis=-1), _softmax(-pk, axis=-1)], axis=-1)
        kv = jnp.einsum("bhsf,bhsd->bhfd", phi_k, v)
        z  = jnp.einsum("bhsf->bhf", phi_k)
        num = jnp.einsum("bhqf,bhfd->bhqd", phi_q, kv)
        den = jnp.einsum("bhqf,bhf->bhq", phi_q, z)[..., None] + 1e-6
        o = num / den
        return (lambda x, *d: x.transpose(*d))(o, 0, 2, 1, 3).reshape(B, S, D) @ wo

    def _B_ref(x, w_gate, w_up, w_down):
        g = jnp.einsum("bsd,df->bsf", x, w_gate)
        u = jnp.einsum("bsd,df->bsf", x, w_up)
        h = g * u
        return jnp.einsum("bsf,fd->bsd", h, w_down)

    x = A_x
    g = _sigmoid((x * gate_w).sum(-1, keepdims=True))
    a = _A_ref(x, A_wqkv, A_w_phi, A_wo)
    b = _B_ref(x, B_w_gate, B_w_up, B_w_down)
    return g * a + (1 - g) * b
```

```python
import functools
import numpy as np
import jax
import jax.numpy as jnp
from jax import lax
import jax.experimental.pallas as pl
import jax.experimental.pallas.tpu as pltpu

S, D, H, DH, F = 2048, 512, 32, 16, 1792
HG = 4
LOG2E = 1.4426950408889634
BF = jnp.bfloat16
F32 = jnp.float32

NT = (((1,), (1,)), ((), ()))
NN = (((1,), (0,)), ((), ()))
TN = (((0,), (0,)), ((), ()))


def _dot(a, b, dims=NN):
    return lax.dot_general(a, b, dims, preferred_element_type=F32)


def _dual_softmax(p):
    parts = [p[8 * f:8 * f + 8] for f in range(DH)]
    mx = functools.reduce(jnp.maximum, parts)
    mn = functools.reduce(jnp.minimum, parts)
    ep = [jnp.exp2(t - mx) for t in parts]
    en = [jnp.exp2(mn - t) for t in parts]
    rp = 1.0 / functools.reduce(jnp.add, ep)
    rn = 1.0 / functools.reduce(jnp.add, en)
    return jnp.concatenate([e * rp for e in ep] + [e * rn for e in en], axis=0)


def make_kernel(T1, T2, FC, unroll1=False, unroll2=False):
    def kernel(x_hbm, wqkv_hbm, wphi_ref, wo_hbm, wg_hbm, wu_hbm, wd_hbm, gw_ref, out_hbm,
               x_v, wqkv_v, wo_v, wg_v, wu_v, wd_v, wall_v, wop_v, phiq_v, g_v, kv_v, z_v, kvb_v, out_v,
               sem_in, sem_x, sem_out):
        n1 = S // T1
        n2 = S // T2
        cp_wqkv = pltpu.make_async_copy(wqkv_hbm, wqkv_v, sem_in.at[0])
        cp_x = [pltpu.make_async_copy(x_hbm.at[pl.ds(i * T1, T1)], x_v.at[pl.ds(i * T1, T1)], sem_x.at[i])
                for i in range(n1)]
        cp_wo = pltpu.make_async_copy(wo_hbm, wo_v, sem_in.at[1])
        cp_wg = pltpu.make_async_copy(wg_hbm, wg_v, sem_in.at[2])
        cp_wu = pltpu.make_async_copy(wu_hbm, wu_v, sem_in.at[3])
        cp_wd = pltpu.make_async_copy(wd_hbm, wd_v, sem_in.at[4])
        cp_wqkv.start()
        for c in cp_x:
            c.start()
        cp_wo.start()
        cp_wg.start()
        cp_wu.start()
        cp_wd.start()

        r = lax.broadcasted_iota(jnp.int32, (128, 128), 0)
        c = lax.broadcasted_iota(jnp.int32, (128, 128), 1)
        head_mask = (r % 8) == (c // 16)
        perm = jnp.where(head_mask & ((r // 8) == (c % 16)), 1.0, 0.0).astype(BF)
        er = lax.broadcasted_iota(jnp.int32, (H, D), 0)
        ec = lax.broadcasted_iota(jnp.int32, (H, D), 1)
        y = _dot(wphi_ref[...], jnp.where(er == ec // DH, 1.0, 0.0).astype(BF))
        yr = lax.broadcasted_iota(jnp.int32, (DH * DH, D), 0)
        yc = lax.broadcasted_iota(jnp.int32, (DH * DH, D), 1)
        y = jnp.where(yr // DH == yc % DH, y, 0.0).astype(BF)
        xr = lax.broadcasted_iota(jnp.int32, (128, DH * DH), 0)
        xc = lax.broadcasted_iota(jnp.int32, (128, DH * DH), 1)
        mall = _dot(jnp.where(xr // 8 == xc % DH, 1.0, 0.0).astype(BF), y)
        cp_wqkv.wait()
        for hg in range(HG):
            m = jnp.where(head_mask, mall[:, hg * 128:(hg + 1) * 128], 0.0).astype(BF)
            for part in range(2):
                w = wqkv_v[:, part * D + hg * 128: part * D + (hg + 1) * 128]
                wall_v[part * D + hg * 128: part * D + (hg + 1) * 128, :] = (_dot(m, w, NT) * LOG2E).astype(BF)
            w = wqkv_v[:, 2 * D + hg * 128: 2 * D + (hg + 1) * 128]
            wall_v[2 * D + hg * 128: 2 * D + (hg + 1) * 128, :] = _dot(perm, w, NT).astype(BF)
        wall_v[3 * D:3 * D + 16, :] = jnp.broadcast_to(gw_ref[...].reshape(1, D), (16, D))
        kv_v[...] = jnp.zeros_like(kv_v)
        z_v[...] = jnp.zeros_like(z_v)

        def phase1(i):
            t0 = pl.multiple_of(i * T1, T1)
            pltpu.make_async_copy(x_hbm.at[pl.ds(t0, T1)], x_v.at[pl.ds(t0, T1)], sem_x.at[i]).wait()
            xb = x_v[pl.ds(t0, T1), :]
            p = _dot(wall_v[...], xb, NT)
            g_v[:, pl.ds(t0, T1)] = jax.nn.sigmoid(p[3 * D:3 * D + 8])
            for hg in range(HG):
                phiq_v[hg * 256:(hg + 1) * 256, pl.ds(t0, T1)] = _dual_softmax(p[hg * 128:(hg + 1) * 128]).astype(BF)
                phik = _dual_softmax(p[D + hg * 128:D + (hg + 1) * 128])
                vt = p[2 * D + hg * 128:2 * D + (hg + 1) * 128].astype(BF)
                kv_v[hg] += _dot(vt, phik.astype(BF), NT)
                z_v[hg] += functools.reduce(jnp.add, [phik[:, j * 128:(j + 1) * 128] for j in range(T1 // 128)])

        if unroll1:
            for i in range(n1):
                phase1(i)
        else:
            pl.loop(0, n1)(phase1)

        r2 = lax.broadcasted_iota(jnp.int32, (128, 256), 0)
        c2 = lax.broadcasted_iota(jnp.int32, (128, 256), 1)
        cp_wo.wait()
        for hg in range(HG):
            kvb_v[hg] = jnp.where((r2 % 8) == (c2 % 8), kv_v[hg], 0.0).astype(BF)
            z_v[hg] = jnp.broadcast_to(jnp.sum(z_v[hg], axis=1, keepdims=True), (256, 128))
            wop_v[hg * 128:(hg + 1) * 128, :] = _dot(perm, wo_v[hg * 128:(hg + 1) * 128, :]).astype(BF)
        cp_wg.wait()
        cp_wu.wait()
        cp_wd.wait()

        def out_copy(i):
            t0 = pl.multiple_of(i * T2, T2)
            return pltpu.make_async_copy(out_v.at[pl.ds(t0, T2)], out_hbm.at[pl.ds(t0, T2)], sem_out.at[i])

        def phase2(i):
            t0 = pl.multiple_of(i * T2, T2)
            xb = x_v[pl.ds(t0, T2), :]
            gt = g_v[:, pl.ds(t0, T2)]
            ots = []
            for hg in range(HG):
                pq = phiq_v[hg * 256:(hg + 1) * 256, pl.ds(t0, T2)]
                num = _dot(kvb_v[hg], pq)
                zz = jnp.concatenate([z_v[hg]] * (T2 // 128), axis=1)
                pz = pq.astype(F32) * zz
                den = functools.reduce(jnp.add, [pz[8 * j:8 * j + 8] for j in range(2 * DH)])
                sc = gt / (den + 1e-6)
                ots.append((num * jnp.concatenate([sc] * DH, axis=0)).astype(BF))
            ot = jnp.concatenate(ots, axis=0)
            a = _dot(ot, wop_v[...], TN)
            b = None
            for j in range(F // FC):
                gg = _dot(xb, wg_v[:, j * FC:(j + 1) * FC])
                uu = _dot(xb, wu_v[:, j * FC:(j + 1) * FC])
                d = _dot((gg * uu).astype(BF), wd_v[j * FC:(j + 1) * FC, :])
                b = d if b is None else b + d
            gtok = jnp.broadcast_to(gt[0:1], (128, T2)).T
            og = 1.0 - gtok
            out_v[pl.ds(t0, T2), :] = (a + jnp.concatenate([og] * (D // 128), axis=1) * b).astype(BF)
            out_copy(i).start()

        if unroll2:
            for i in range(n2):
                phase2(i)
        else:
            pl.loop(0, n2)(phase2)
        for i in range(n2):
            out_copy(i).wait()
    return kernel


def build(T1=256, T2=256, FC=1792, unroll1=False, unroll2=False, vmem=100):
    @jax.jit
    def fn(A_x, A_wqkv, A_w_phi, A_wo, B_x, B_w_gate, B_w_up, B_w_down, gate_w):
        any_spec = pl.BlockSpec(memory_space=pl.ANY)
        vm = pl.BlockSpec(memory_space=pltpu.VMEM)
        out = pl.pallas_call(
            make_kernel(T1, T2, FC, unroll1, unroll2),
            in_specs=[any_spec, any_spec, vm, any_spec, any_spec, any_spec, any_spec, vm],
            out_specs=any_spec,
            out_shape=jax.ShapeDtypeStruct((S, D), BF),
            scratch_shapes=[
                pltpu.VMEM((S, D), BF), pltpu.VMEM((D, 3 * D), BF), pltpu.VMEM((D, D), BF),
                pltpu.VMEM((D, F), BF), pltpu.VMEM((D, F), BF), pltpu.VMEM((F, D), BF),
                pltpu.VMEM((3 * D + 16, D), BF), pltpu.VMEM((D, D), BF),
                pltpu.VMEM((2 * D, S), BF), pltpu.VMEM((8, S), F32),
                pltpu.VMEM((HG, 128, 256), F32), pltpu.VMEM((HG, 256, 128), F32), pltpu.VMEM((HG, 128, 256), BF),
                pltpu.VMEM((S, D), BF),
                pltpu.SemaphoreType.DMA((5,)), pltpu.SemaphoreType.DMA((S // T1,)), pltpu.SemaphoreType.DMA((S // T2,)),
            ],
            compiler_params=pltpu.CompilerParams(vmem_limit_bytes=vmem * 1024 * 1024),
        )(A_x.reshape(S, D), A_wqkv, A_w_phi.transpose(1, 2, 0).reshape(DH * DH, H), A_wo, B_w_gate, B_w_up, B_w_down, gate_w)
        return out.reshape(1, S, D)
    return fn


pallas_gated_mix__linear_kernel_hedgehog__glu_gated_bilinear__prompt_kernel = build(**dict(T1=512,T2=512))
```

```python
import functools
import jax
import jax.numpy as jnp
from jax import lax
import jax.experimental.pallas as pl
import jax.experimental.pallas.tpu as pltpu

S, D, H, DH, F = 2048, 512, 32, 16, 1792
HS, HD, HF = S // 2, D // 2, F // 2
NG = 8
WR = 3 * HD + 16
LOG2E = 1.4426950408889634
BF = jnp.bfloat16
F32 = jnp.float32

NT = (((1,), (1,)), ((), ()))
NN = (((1,), (0,)), ((), ()))
TN = (((0,), (0,)), ((), ()))


def _dot(a, b, dims=NN):
    return lax.dot_general(a, b, dims, preferred_element_type=F32)


def _red(op, parts):
    r = functools.reduce(op, parts)
    return op(r, pltpu.roll(r, 4, 0))


def _dual_softmax(p):
    parts = [p[8 * i:8 * i + 8] for i in range(8)]
    mx = _red(jnp.maximum, parts)
    mn = _red(jnp.minimum, parts)
    ep = [jnp.exp2(t - mx) for t in parts]
    en = [jnp.exp2(mn - t) for t in parts]
    rp = 1.0 / _red(jnp.add, ep)
    rn = 1.0 / _red(jnp.add, en)
    return jnp.concatenate([e * rp for e in ep] + [e * rn for e in en], axis=0)


def _sum(a, b, sgn=1):
    a = a.astype(F32)
    b = b.astype(F32)
    return (a + b if sgn > 0 else a - b).astype(BF)


def _a_ops(a11, a12, a21, a22):
    return [_sum(a11, a22), _sum(a21, a22), a11.astype(BF), a22.astype(BF),
            _sum(a11, a12), _sum(a21, a11, -1), _sum(a12, a22, -1)]


def _b_ops(b11, b12, b21, b22):
    return [_sum(b11, b22), b11.astype(BF), _sum(b12, b22, -1), _sum(b21, b11, -1),
            b22.astype(BF), _sum(b11, b12), _sum(b21, b22)]


def _combine(m):
    m1, m2, m3, m4, m5, m6, m7 = m
    return (m1 + m4) + (m7 - m5), m3 + m5, m2 + m4, (m1 - m2) + (m3 + m6)


ORDER = (2, 3, 0, 1, 4, 5, 6)


def _iota(shape, axis):
    return lax.broadcasted_iota(jnp.int32, shape, axis)


def make_kernel(T1, T2, FC, TO, RC, AST, PLAN, SLOTS):
    n1, n2, no = HS // T1, HS // T2, T2 // TO

    def kernel(x_hbm, wqkv_hbm, wphi_hbm, wo_hbm, wg_hbm, wu_hbm, wd_hbm, gw_hbm, out_hbm, wphi_ref, gw_ref,
               x_v, wqkv_v, wo_v, wg_v, wu_v, wd_v, wall_v, xs_v, kv_v, z_v, out_v,
               sem_in, sem_x, sem_out):
        def x_copy(i, half):
            t0 = pl.multiple_of(half * HS + i * T1, T1)
            return pltpu.make_async_copy(x_hbm.at[pl.ds(t0, T1)], x_v.at[pl.ds(t0, T1)], sem_x.at[half, i])

        cp_w = [pltpu.make_async_copy(wqkv_hbm.at[:, pl.ds(p * D, D)], wqkv_v.at[:, pl.ds(p * D, D)], sem_in.at[p])
                for p in range(3)]
        cp_rest = [pltpu.make_async_copy(wg_hbm, wg_v, sem_in.at[3]), pltpu.make_async_copy(wu_hbm, wu_v, sem_in.at[4]),
                   pltpu.make_async_copy(wd_hbm, wd_v, sem_in.at[5]), pltpu.make_async_copy(wo_hbm, wo_v, sem_in.at[6])]
        cp_phi = pltpu.make_async_copy(wphi_hbm, wphi_ref, sem_in.at[7])
        cp_gw = pltpu.make_async_copy(gw_hbm, gw_ref, sem_in.at[8])
        cps = dict(p=[cp_phi], g=[cp_gw], q=[cp_w[0]], k=[cp_w[1]], v=[cp_w[2]],
                   G=[cp_rest[0]], U=[cp_rest[1]], D=[cp_rest[2]], O=[cp_rest[3]])
        for i in range(n1):
            cps[str(i)] = [x_copy(i, 0), x_copy(i, 1)]
        stages = iter(PLAN.split('|'))

        def start_stage():
            for name in next(stages):
                for cp in cps[name]:
                    cp.start()

        start_stage()
        cp_phi.wait()

        y = _dot(wphi_ref[...], jnp.where(_iota((H, D), 0) == _iota((H, D), 1) // DH, 1.0, 0.0).astype(BF))
        y = jnp.where(_iota((DH * DH, D), 0) // DH == _iota((DH * DH, D), 1) % DH, y, 0.0).astype(BF)
        sel = (_iota((128, DH * DH), 0) % 64) // 4 == _iota((128, DH * DH), 1) % DH
        mall = _dot(jnp.where(sel, 1.0, 0.0).astype(BF), y)
        r, c = _iota((128, 128), 0), _iota((128, 128), 1)
        head_mask = (r // 64) * 4 + r % 4 == c // DH
        ms = [jnp.where(head_mask, mall[:, j * 128:(j + 1) * 128], 0.0).astype(BF) for j in range(4)]

        def prep(part, j):
            w1 = wqkv_v[:, part * D + j * 128: part * D + (j + 1) * 128]
            w2 = wqkv_v[:, part * D + HD + j * 128: part * D + HD + (j + 1) * 128]
            if part < 2:
                w1 = _dot(ms[j], w1, NT) * LOG2E
                w2 = _dot(ms[2 + j], w2, NT) * LOG2E
            else:
                w1, w2 = w1.T, w2.T
            slot = (2, 0, 1)[part] * HD + j * 128
            for q, w in enumerate(_b_ops(w1[:, :HD], w2[:, :HD], w1[:, HD:], w2[:, HD:])):
                wall_v[q, slot:slot + 128, :] = w

        cp_w[2].wait()
        start_stage()
        prep(2, 0)
        prep(2, 1)
        cp_w[1].wait()
        start_stage()
        cp_gw.wait()
        gw = jnp.broadcast_to(gw_ref[...].reshape(1, D), (16, D))
        zero = jnp.zeros((16, HD), BF)
        for q, w in enumerate(_b_ops(gw[:, :HD], zero, gw[:, HD:], zero)):
            wall_v[q, 3 * HD:, :] = w
        prep(1, 0)
        prep(1, 1)

        def x_ops(i):
            lo, hi = pl.ds(i * T1, T1), pl.ds(HS + i * T1, T1)
            x_copy(i, 0).wait()
            x_copy(i, 1).wait()
            start_stage()
            xa = _a_ops(x_v[lo, :HD], x_v[lo, HD:], x_v[hi, :HD], x_v[hi, HD:])
            for q in range(7):
                xs_v[q, lo, :] = xa[q]
            return xa

        def project(rows, xa, jobs):
            m = {}
            for n, q in enumerate(ORDER):
                m[q] = _dot(wall_v[q, rows], xa[q], NT)
                if jobs and n in SLOTS:
                    accumulate(*jobs.pop(0))
            return _combine([m[q] for q in range(7)])

        def accumulate(i, ks, vs, o, half):
            hq = half * (NG // 2) + o // 64
            phik = _dual_softmax(jnp.concatenate([ks[half][o:o + 64], ks[2 + half][o:o + 64]], axis=1))
            vt = jnp.concatenate([vs[half][o:o + 64], vs[2 + half][o:o + 64]], axis=1)
            kv = _dot(vt.astype(BF), phik.astype(BF), NT)
            z = functools.reduce(jnp.add, [phik[:, j * 128:(j + 1) * 128] for j in range(2 * T1 // 128)])
            kv_v[hq] = kv if i == 0 else kv_v[hq] + kv
            z_v[hq] = z if i == 0 else z_v[hq] + z

        jobs = []
        for i in range(n1):
            if i == n1 - 1:
                cp_w[0].wait()
            xa = x_ops(i)
            ks = project(slice(0, HD), xa, jobs)
            vs = project(slice(HD, 2 * HD), xa, jobs)
            assert not jobs
            jobs = [(i, ks, vs, o, half) for o in range(0, HD, 64) for half in range(2)]
        for n, job in enumerate(jobs):
            accumulate(*job)
            if n in (3, 5):
                prep(0, (n - 3) // 2)

        for cp in cp_rest:
            cp.wait()

        def out_copy(i, j, half):
            t0 = pl.multiple_of(half * HS + i * T2 + j * TO, TO)
            return pltpu.make_async_copy(out_v.at[pl.ds(t0, TO)], out_hbm.at[pl.ds(t0, TO)], sem_out.at[half, i * no + j])

        @pl.loop(0, n2)
        def _(i):
            lo = pl.ds(pl.multiple_of(i * T2, T2), T2)
            xa = [xs_v[q, lo, :] for q in range(7)]
            qs = _combine([_dot(wall_v[q, 2 * HD:], xa[q], NT) for q in range(7)])
            gts = [jax.nn.sigmoid(qs[0][HD:HD + 8]), jax.nn.sigmoid(qs[2][HD:HD + 8])]
            kmask = _iota((64, 128), 0) // DH == _iota((64, 128), 1) % 4

            def attend(hq):
                kvb = jnp.where(kmask, kv_v[hq], 0.0).astype(BF)
                zb = jnp.sum(z_v[hq], axis=1, keepdims=True)
                o = (hq % (NG // 2)) * 64
                res = []
                for half in range(2):
                    phi = _dual_softmax(qs[2 * half + hq // (NG // 2)][o:o + 64])
                    num = _dot(kvb, phi.astype(BF))
                    pz = phi * zb
                    den = _red(jnp.add, [pz[8 * k:8 * k + 8] for k in range(DH)])
                    sc = gts[half] / (den + 1e-6)
                    res.append(num * jnp.concatenate(
                        [jnp.broadcast_to(sc[k:k + 1], (DH, T2)) for k in range(4)], axis=0))
                return res

            oas = []
            md = [None] * 7
            for j in range(HF // FC):
                hs = []
                for half in range(2):
                    cs = slice(half * HF + j * FC, half * HF + (j + 1) * FC)
                    wb = _b_ops(wg_v[:HD, cs], wu_v[:HD, cs], wg_v[HD:, cs], wu_v[HD:, cs])
                    g1, u1, g2, u2 = _combine([_dot(p, q) for p, q in zip(xa, wb)])
                    hs.append((g1 * u1, g2 * u2))
                    step = 2 * j + half
                    if step % AST == 0 and step // AST < NG:
                        k = step // AST
                        if k % 2 == 0:
                            o1 = attend(k // 2)
                        else:
                            o2 = attend(NG // 2 + k // 2)
                            oas.append(_a_ops(o1[0], o2[0], o1[1], o2[1]))
                ha = _a_ops(hs[0][0], hs[1][0], hs[0][1], hs[1][1])
                r1, r2 = slice(j * FC, (j + 1) * FC), slice(HF + j * FC, HF + (j + 1) * FC)
                wb = _b_ops(wd_v[r1, :HD], wd_v[r1, HD:], wd_v[r2, :HD], wd_v[r2, HD:])
                for q in range(7):
                    d = _dot(ha[q], wb[q])
                    md[q] = d if md[q] is None else md[q] + d
            b = _combine(md)
            oa = [jnp.concatenate([t[q] for t in oas], axis=0) for q in range(7)]
            ob = _b_ops(wo_v[:HD, :HD], wo_v[:HD, HD:], wo_v[HD:, :HD], wo_v[HD:, HD:])
            ogf = [1.0 - jnp.broadcast_to(g[0:1], (128, T2)).T for g in gts]
            for j in range(no):
                rows = [pl.ds(pl.multiple_of(half * HS + i * T2 + j * TO, TO), TO) for half in range(2)]
                ogs = [jnp.concatenate([g[j * TO:(j + 1) * TO]] * (HD // 128), axis=1) for g in ogf]
                a = _combine([_dot(p[:, j * TO:(j + 1) * TO], q, TN) for p, q in zip(oa, ob)])
                js = slice(j * TO, (j + 1) * TO)
                for half in range(2):
                    out_v[rows[half], :HD] = (a[2 * half] + ogs[half] * b[2 * half][js]).astype(BF)
                    out_v[rows[half], HD:] = (a[2 * half + 1] + ogs[half] * b[2 * half + 1][js]).astype(BF)
                    out_copy(i, j, half).start()

        for i in range(n2):
            for j in range(no):
                for half in range(2):
                    out_copy(i, j, half).wait()
    return kernel


def build(T1=256, T2=512, FC=128, TO=256, RC=256, AST=1, SLOTS=(0,2,4,5), PLAN='pvkg|0|1|23qGUDO|||', vmem=100):
    @jax.jit
    def fn(A_x, A_wqkv, A_w_phi, A_wo, B_x, B_w_gate, B_w_up, B_w_down, gate_w):
        any_spec = pl.BlockSpec(memory_space=pl.ANY)
        out = pl.pallas_call(
            make_kernel(T1, T2, FC, TO, RC, AST, PLAN, SLOTS),
            in_specs=[any_spec] * 8,
            out_specs=any_spec,
            out_shape=jax.ShapeDtypeStruct((S, D), BF),
            scratch_shapes=[
                pltpu.VMEM((DH * DH, H), BF), pltpu.VMEM((D,), BF),
                pltpu.VMEM((S, D), BF), pltpu.VMEM((D, 3 * D), BF), pltpu.VMEM((D, D), BF),
                pltpu.VMEM((D, F), BF), pltpu.VMEM((D, F), BF), pltpu.VMEM((F, D), BF),
                pltpu.VMEM((7, WR, HD), BF), pltpu.VMEM((7, HS, HD), BF),
                pltpu.VMEM((NG, 64, 128), F32), pltpu.VMEM((NG, 128, 128), F32),
                pltpu.VMEM((S, D), BF),
                pltpu.SemaphoreType.DMA((9,)), pltpu.SemaphoreType.DMA((2, HS // T1)), pltpu.SemaphoreType.DMA((2, HS // TO)),
            ],
            compiler_params=pltpu.CompilerParams(vmem_limit_bytes=vmem * 1024 * 1024),
        )(A_x.reshape(S, D), A_wqkv, A_w_phi.transpose(1, 2, 0).reshape(DH * DH, H), A_wo,
          B_w_gate, B_w_up, B_w_down, gate_w)
        return out.reshape(1, S, D)
    return fn


pallas_gated_mix__linear_kernel_hedgehog__glu_gated_bilinear__prompt_kernel = build(**dict())
```
